```python
import os as _os
_os.environ.setdefault("JAX_PLATFORMS", "cpu")
import jax
import jax.numpy as jnp

def _softmax(x, axis=-1):
    return jax.nn.softmax(x, axis=axis)
def _gelu(x):
    return jax.nn.gelu(x, approximate=True)
def _silu(x):
    return jax.nn.silu(x)
def _sigmoid(x):
    return jax.nn.sigmoid(x)
def _layernorm(x, axis=-1, eps=1e-5):
    m = jnp.mean(x, axis=axis, keepdims=True)
    v = jnp.var(x, axis=axis, keepdims=True)
    return (x - m) / jnp.sqrt(v + eps)
def _scatter_add(tgt, idx, src, axis=0):
    return tgt.at[idx].add(src)
def _segment_sum(src, seg, n):
    return jax.ops.segment_sum(src, seg, n)
class _Rng:
    def __init__(self, key):
        self._k = key
    def _next(self):
        self._k, sub = jax.random.split(self._k)
        return sub
    def normal(self, shape):
        return jax.random.normal(self._next(), shape, dtype=jnp.bfloat16)
    def randint(self, lo, hi, shape):
        return jax.random.randint(self._next(), shape, lo, hi, dtype=jnp.int32)
    def uniform(self, shape, lo=0.0, hi=1.0):
        return jax.random.uniform(self._next(), shape, jnp.bfloat16, lo, hi)
    def permutation(self, n):
        return jax.random.permutation(self._next(), n)


kernel_name = 'interleave_layers__mha_block__dense_activation_mish__prompt'

def setup_inputs():
    _rng = _Rng(jax.random.key(int.from_bytes(__import__("os").urandom(4), "little")))
    _w = (lambda a: (lambda t: t.astype(jnp.bfloat16) if jnp.issubdtype(t.dtype, jnp.floating) else t)(jnp.asarray(a)))
    def _A_setup():
        B, S, D, H = 1, 2048, 512, 32
        return {
            "x": _w((lambda *s: _rng.normal(s) * 0.05)(B, S, D)),
            "wqkv": _w((lambda *s: _rng.normal(s) * 0.05)(D, 3 * D)),
            "wo": _w((lambda *s: _rng.normal(s) * 0.05)(D, D)),
        }
    _A_in = _A_setup()

    def _B_setup():
        B, S, D, F = 1, 2048, 512, 1792
        return {
            "x": _w((lambda *s: _rng.normal(s) * 0.05)(B, S, D)),
            "w1": _w((lambda *s: _rng.normal(s) * 0.4)(D, F) * (D ** -0.5)),
            "b1": _w((lambda *s: _rng.normal(s) * 0.4)(F)),
            "w2": _w((lambda *s: _rng.normal(s) * 0.4)(F, D) * (F ** -0.5)),
        }
    _B_in = _B_setup()

    return {
        "A_x": _A_in["x"],
        "A_wqkv": _A_in["wqkv"],
        "A_wo": _A_in["wo"],
        "B_x": _B_in["x"],
        "B_w1": _B_in["w1"],
        "B_b1": _B_in["b1"],
        "B_w2": _B_in["w2"],
    }

def reference(A_x, A_wqkv, A_wo, B_x, B_w1, B_b1, B_w2):
    def _A_ref(x, wqkv, wo):
        B, S, D = x.shape
        H = 32
        Dh = D // H
        qkv = (lambda x, *d: x.transpose(*d))((x @ wqkv).reshape(B, S, 3, H, Dh), 2, 0, 3, 1, 4)
        q, k, v = qkv[0], qkv[1], qkv[2]
        scores = jnp.einsum("bhqd,bhkd->bhqk", q, k) * (Dh ** -0.5)
        p = _softmax(scores, axis=-1)
        o = jnp.einsum("bhqk,bhkd->bhqd", p, v)
        return (lambda x, *d: x.transpose(*d))(o, 0, 2, 1, 3).reshape(B, S, D) @ wo

    def _B_ref(x, w1, b1, w2):
        h = jnp.einsum("bsd,df->bsf", x, w1) + b1
        sp = jnp.log1p(jnp.exp(-jnp.abs(h))) + jnp.where(h > 0, h, jnp.zeros_like(h))
        act = h * jnp.tanh(sp)
        return jnp.einsum("bsf,fd->bsd", act, w2)

    x = A_x
    x = x + _A_ref(_layernorm(x, axis=-1), A_wqkv, A_wo)
    x = x + _B_ref(_layernorm(x, axis=-1), B_w1, B_b1, B_w2)
    x = x + _A_ref(_layernorm(x, axis=-1), A_wqkv, A_wo)
    x = x + _B_ref(_layernorm(x, axis=-1), B_w1, B_b1, B_w2)
    return x
```

```python
import functools
import math

import jax
import jax.numpy as jnp
import jax.experimental.pallas as pl
import jax.experimental.pallas.tpu as pltpu

S, D, H, DH, F = 2048, 512, 32, 16, 1792
EPS = 1e-5
QSCALE = (DH ** -0.5) * math.log2(math.e)

TQ = 512
KS = 128
LAG = 3
NQ = S // TQ
NU = H * NQ
NP = S // KS
RB = 256
NRB = S // RB

f32 = jnp.float32
bf16 = jnp.bfloat16


def _ln(x):
    mu = jnp.mean(x, axis=-1, keepdims=True)
    xc = x - mu
    var = jnp.mean(xc * xc, axis=-1, keepdims=True)
    return xc * jax.lax.rsqrt(var + EPS)


def _mish(h):
    sp = jnp.log1p(jnp.exp(-jnp.abs(h))) + jnp.maximum(h, 0.0)
    return h * jnp.tanh(sp)


def _kernel(x_ref, wqvt_ref, wk_ref, wo_ref, w1_ref, b1_ref, w2_ref, out_ref,
            xs_ref, qt_ref, vt_ref, k_ref, ot_ref, sa_ref, sb_ref):

    def qkv_block(r0, x):
        hb = _ln(x).astype(bf16)
        qvt = jax.lax.dot_general(wqvt_ref[...], hb, (((1,), (1,)), ((), ())),
                                  preferred_element_type=f32)
        qt_ref[:, pl.ds(r0, RB)] = (qvt[:D] * QSCALE).astype(bf16)
        vt_ref[:, pl.ds(r0, RB)] = qvt[D:].astype(bf16)
        kb = jnp.dot(hb, wk_ref[...], preferred_element_type=f32).astype(bf16)
        for h in range(H):
            k_ref[h, pl.ds(r0, RB), :] = kb[:, h * DH:(h + 1) * DH]

    def p1_piece(u, j, s_ref, m8):
        h = u // NQ
        qi = u % NQ
        r0 = pl.multiple_of(h * DH, DH)
        q0 = pl.multiple_of(qi * TQ, TQ)
        qt = qt_ref[pl.ds(r0, DH), pl.ds(q0, TQ)]
        s = jnp.dot(k_ref[h, j * KS:(j + 1) * KS, :], qt, preferred_element_type=f32)
        s_ref[j * KS:(j + 1) * KS, :] = s
        return jnp.maximum(m8, s.reshape(KS // 8, 8, TQ).max(axis=0))

    def p2_piece(u, j, s_ref, m, l8, acc):
        h = u // NQ
        r0 = pl.multiple_of(h * DH, DH)
        p = jnp.exp2(s_ref[j * KS:(j + 1) * KS, :] - m)
        l8 = l8 + p.reshape(KS // 8, 8, TQ).sum(axis=0)
        acc = acc + jnp.dot(vt_ref[pl.ds(r0, DH), j * KS:(j + 1) * KS], p.astype(bf16),
                            preferred_element_type=f32)
        return l8, acc

    def finalize(u, l8, acc):
        l = l8.sum(axis=0, keepdims=True)
        h = u // NQ
        qi = u % NQ
        r0 = pl.multiple_of(h * DH, DH)
        q0 = pl.multiple_of(qi * TQ, TQ)
        ot_ref[pl.ds(r0, DH), pl.ds(q0, TQ)] = (acc / l).astype(bf16)

    def attention():
        minit = jnp.full((8, TQ), -jnp.inf, f32)
        zl = jnp.zeros((8, TQ), f32)
        za = jnp.zeros((DH, TQ), f32)
        m8 = minit
        for j in range(NP):
            m8 = p1_piece(0, j, sa_ref, m8)
        sb_ref[(NP - LAG) * KS:, :] = jnp.zeros((LAG * KS, TQ), f32)

        def unit(u, carry, cur_ref, nxt_ref):
            m8_cur, m_prev, l8p, accp = carry
            m = m8_cur.max(axis=0, keepdims=True)
            un = jnp.minimum(u + 1, NU - 1)
            up = jnp.maximum(u - 1, 0)
            m8n = minit
            l8 = zl
            acc = za
            for j in range(NP):
                m8n = p1_piece(un, j, nxt_ref, m8n)
                if j < LAG:
                    l8p, accp = p2_piece(up, NP - LAG + j, nxt_ref, m_prev, l8p, accp)
                    if j == LAG - 1:
                        finalize(up, l8p, accp)
                else:
                    l8, acc = p2_piece(u, j - LAG, cur_ref, m, l8, acc)
            return m8n, m, l8, acc

        def pair(i, carry):
            carry = unit(2 * i, carry, sa_ref, sb_ref)
            carry = unit(2 * i + 1, carry, sb_ref, sa_ref)
            return carry

        carry = jax.lax.fori_loop(0, NU // 2, pair, (m8, jnp.zeros((1, TQ), f32), zl, za))
        _, m, l8, acc = carry
        for j in range(LAG):
            l8, acc = p2_piece(NU - 1, NP - LAG + j, sb_ref, m, l8, acc)
        finalize(NU - 1, l8, acc)

    def post_block(r0):
        ob = ot_ref[:, pl.ds(r0, RB)].T
        x = xs_ref[pl.ds(r0, RB), :] + jnp.dot(ob, wo_ref[...], preferred_element_type=f32)
        hb = _ln(x).astype(bf16)
        h1 = jnp.dot(hb, w1_ref[...], preferred_element_type=f32) + b1_ref[...].astype(f32)
        a = _mish(h1).astype(bf16)
        return x + jnp.dot(a, w2_ref[...], preferred_element_type=f32)

    def phase0(i, _):
        r0 = pl.multiple_of(i * RB, RB)
        x = x_ref[pl.ds(r0, RB), :].astype(f32)
        xs_ref[pl.ds(r0, RB), :] = x
        qkv_block(r0, x)
        return 0

    def phase1(i, _):
        r0 = pl.multiple_of(i * RB, RB)
        x = post_block(r0)
        xs_ref[pl.ds(r0, RB), :] = x
        qkv_block(r0, x)
        return 0

    def phase2(i, _):
        r0 = pl.multiple_of(i * RB, RB)
        out_ref[pl.ds(r0, RB), :] = post_block(r0).astype(out_ref.dtype)
        return 0

    jax.lax.fori_loop(0, NRB, phase0, 0)
    attention()
    jax.lax.fori_loop(0, NRB, phase1, 0)
    attention()
    jax.lax.fori_loop(0, NRB, phase2, 0)


@jax.jit
def pallas_interleave_layers__mha_block__dense_activation_mish__prompt_kernel(
    A_x: jax.Array,
    A_wqkv: jax.Array,
    A_wo: jax.Array,
    B_x: jax.Array,
    B_w1: jax.Array,
    B_b1: jax.Array,
    B_w2: jax.Array,
):
    x = A_x.reshape(S, D)
    wqvt = jnp.concatenate([A_wqkv[:, :D], A_wqkv[:, 2 * D:]], axis=1).T
    wk = A_wqkv[:, D:2 * D]
    b1 = B_b1.reshape(1, F)
    out = pl.pallas_call(
        _kernel,
        out_shape=jax.ShapeDtypeStruct((S, D), A_x.dtype),
        scratch_shapes=[
            pltpu.VMEM((S, D), f32),
            pltpu.VMEM((D, S), bf16),
            pltpu.VMEM((D, S), bf16),
            pltpu.VMEM((H, S, DH), bf16),
            pltpu.VMEM((D, S), bf16),
            pltpu.VMEM((S, TQ), f32),
            pltpu.VMEM((S, TQ), f32),
        ],
        compiler_params=pltpu.CompilerParams(vmem_limit_bytes=110 * 1024 * 1024),
        name="mha_mish_layers",
    )(x, wqvt, wk, A_wo, B_w1, b1, B_w2)
    return out.reshape(1, S, D)
```

```python
import functools
import math

import jax
import jax.numpy as jnp
import jax.experimental.pallas as pl
import jax.experimental.pallas.tpu as pltpu

S, D, H, DH, F = 2048, 512, 32, 16, 1792
EPS = 1e-5
QSCALE = (DH ** -0.5) * math.log2(math.e)

TQ = 512
KS = 128
LAG = 3
TOK = 3
NQ = S // TQ
NU = H * NQ
NP = S // KS
RB = 256
NRB = S // RB

f32 = jnp.float32
bf16 = jnp.bfloat16


def _ln(x):
    mu = jnp.mean(x, axis=-1, keepdims=True)
    xc = x - mu
    var = jnp.mean(xc * xc, axis=-1, keepdims=True)
    return xc * jax.lax.rsqrt(var + EPS)


def _mish(h):
    sp = jnp.log1p(jnp.exp(-jnp.abs(h))) + jnp.maximum(h, 0.0)
    return h * jnp.tanh(sp)


def _kernel(x_ref, wqkv_ref, wo_hbm, w1_hbm, b1_ref, w2_hbm, out_ref,
            xs_ref, qt_ref, vt_ref, k_ref, ot_ref, sa_ref, sb_ref,
            wqvt_ref, wo_ref, w1_ref, w2_ref, sems):
    cp_wo = pltpu.make_async_copy(wo_hbm, wo_ref, sems.at[0])
    cp_w1 = pltpu.make_async_copy(w1_hbm, w1_ref, sems.at[1])
    cp_w2 = pltpu.make_async_copy(w2_hbm, w2_ref, sems.at[2])
    cp_wo.start()
    cp_w1.start()
    cp_w2.start()
    wqvt_ref[0:D, :] = wqkv_ref[:, 0:D].T
    wqvt_ref[D:2 * D, :] = wqkv_ref[:, 2 * D:3 * D].T

    def rows(i):
        return pl.ds(pl.multiple_of(i * RB, RB), RB)

    def st_qkv(i, hb):
        kb = jnp.dot(hb, wqkv_ref[:, D:2 * D], preferred_element_type=f32).astype(bf16)
        for h in range(H):
            k_ref[h, rows(i), :] = kb[:, h * DH:(h + 1) * DH]
        qvt = jax.lax.dot_general(wqvt_ref[...], hb, (((1,), (1,)), ((), ())),
                                  preferred_element_type=f32)
        qt_ref[:, rows(i)] = (qvt[:D] * QSCALE).astype(bf16)
        vt_ref[:, rows(i)] = qvt[D:].astype(bf16)

    def st_in(i):
        x = x_ref[0, rows(i), :].astype(f32)
        xs_ref[rows(i), :] = x
        return _ln(x).astype(bf16)

    def st_oproj(i):
        ob = ot_ref[:, rows(i)].T
        x = xs_ref[rows(i), :] + jnp.dot(ob, wo_ref[...], preferred_element_type=f32)
        xs_ref[rows(i), :] = x
        return _ln(x).astype(bf16)

    def st_mlp(i, hb, last):
        h1 = jnp.dot(hb, w1_ref[...], preferred_element_type=f32) + b1_ref[...].astype(f32)
        a = _mish(h1).astype(bf16)
        x = xs_ref[rows(i), :] + jnp.dot(a, w2_ref[...], preferred_element_type=f32)
        if last:
            out_ref[0, rows(i), :] = x.astype(out_ref.dtype)
            return None
        xs_ref[rows(i), :] = x
        return _ln(x).astype(bf16)

    def p1_piece(u, j, s_ref, m8):
        h = u // NQ
        qi = u % NQ
        r0 = pl.multiple_of(h * DH, DH)
        q0 = pl.multiple_of(qi * TQ, TQ)
        qt = qt_ref[pl.ds(r0, DH), pl.ds(q0, TQ)]
        s = jnp.dot(k_ref[h, j * KS:(j + 1) * KS, :], qt, preferred_element_type=f32)
        s_ref[j * KS:(j + 1) * KS, :] = s
        return jnp.maximum(m8, s.reshape(KS // 8, 8, TQ).max(axis=0))

    def p2_piece(u, j, s_ref, m, l8, acc):
        h = u // NQ
        r0 = pl.multiple_of(h * DH, DH)
        p = jnp.exp2(s_ref[j * KS:(j + 1) * KS, :] - m)
        for i in reversed(range(KS // 8)):
            l8 = l8 + p[8 * i:8 * i + 8, :]
        acc = acc + jnp.dot(vt_ref[pl.ds(r0, DH), j * KS:(j + 1) * KS], p.astype(bf16),
                            preferred_element_type=f32)
        return l8, acc

    def finalize(u, l8, acc):
        l = l8.sum(axis=0, keepdims=True)
        h = u // NQ
        qi = u % NQ
        r0 = pl.multiple_of(h * DH, DH)
        q0 = pl.multiple_of(qi * TQ, TQ)
        ot_ref[pl.ds(r0, DH), pl.ds(q0, TQ)] = (acc / l).astype(bf16)

    def attention():
        minit = jnp.full((8, TQ), -jnp.inf, f32)
        zl = jnp.zeros((8, TQ), f32)
        za = jnp.zeros((DH, TQ), f32)
        m8 = minit
        for j in range(NP):
            m8 = p1_piece(0, j, sa_ref, m8)
        sb_ref[(NP - LAG) * KS:, :] = jnp.zeros((LAG * KS, TQ), f32)

        def unit(u, carry, cur_ref, nxt_ref):
            m8_cur, m_prev, l8p, accp = carry
            m = m8_cur.max(axis=0, keepdims=True)
            un = jnp.minimum(u + 1, NU - 1)
            up = jnp.maximum(u - 1, 0)
            m8n = minit
            l8 = zl
            acc = za
            hist = []

            def tok(mm, j):
                if j - TOK < 0:
                    return mm
                t = hist[j - TOK][0:1, :]
                return jnp.maximum(mm, jnp.minimum(mm, t))

            for j in range(NP):
                m8n = p1_piece(un, j, nxt_ref, m8n)
                hist.append(m8n)
                if j < LAG:
                    l8p, accp = p2_piece(up, NP - LAG + j, nxt_ref, tok(m_prev, j), l8p, accp)
                    if j == LAG - 1:
                        finalize(up, l8p, accp)
                else:
                    l8, acc = p2_piece(u, j - LAG, cur_ref, tok(m, j), l8, acc)
            return m8n, m, l8, acc

        def pair(i, carry):
            carry = unit(2 * i, carry, sa_ref, sb_ref)
            carry = unit(2 * i + 1, carry, sb_ref, sa_ref)
            return carry

        carry = jax.lax.fori_loop(0, NU // 2, pair, (m8, jnp.zeros((1, TQ), f32), zl, za))
        _, m, l8, acc = carry
        for j in range(LAG):
            l8, acc = p2_piece(NU - 1, NP - LAG + j, sb_ref, m, l8, acc)
        finalize(NU - 1, l8, acc)

    def phase_first():
        h = st_in(0)

        def body(i, h):
            hn = st_in(i + 1)
            st_qkv(i, h)
            return hn

        h = jax.lax.fori_loop(0, NRB - 1, body, h)
        st_qkv(NRB - 1, h)

    def phase_mid():
        h2 = st_oproj(0)
        h1 = st_mlp(0, h2, False)
        h2 = st_oproj(1)

        def body(i, carry):
            h2, h1 = carry
            h1n = st_mlp(i, h2, False)
            h2n = st_oproj(i + 1)
            st_qkv(i - 1, h1)
            return h2n, h1n

        h2, h1 = jax.lax.fori_loop(1, NRB - 1, body, (h2, h1))
        h1n = st_mlp(NRB - 1, h2, False)
        st_qkv(NRB - 2, h1)
        st_qkv(NRB - 1, h1n)

    def phase_last():
        h2 = st_oproj(0)

        def body(i, h2):
            st_mlp(i, h2, True)
            return st_oproj(i + 1)

        h2 = jax.lax.fori_loop(0, NRB - 1, body, h2)
        st_mlp(NRB - 1, h2, True)

    phase_first()
    attention()
    cp_wo.wait()
    cp_w1.wait()
    cp_w2.wait()
    phase_mid()
    attention()
    phase_last()


@jax.jit
def pallas_interleave_layers__mha_block__dense_activation_mish__prompt_kernel(
    A_x: jax.Array,
    A_wqkv: jax.Array,
    A_wo: jax.Array,
    B_x: jax.Array,
    B_w1: jax.Array,
    B_b1: jax.Array,
    B_w2: jax.Array,
):
    b1 = B_b1.reshape(1, F)
    vmem = pl.BlockSpec(memory_space=pltpu.VMEM)
    hbm = pl.BlockSpec(memory_space=pl.ANY)
    out = pl.pallas_call(
        _kernel,
        out_shape=jax.ShapeDtypeStruct((1, S, D), A_x.dtype),
        in_specs=[vmem, vmem, hbm, hbm, vmem, hbm],
        out_specs=vmem,
        scratch_shapes=[
            pltpu.VMEM((S, D), f32),
            pltpu.VMEM((D, S), bf16),
            pltpu.VMEM((D, S), bf16),
            pltpu.VMEM((H, S, DH), bf16),
            pltpu.VMEM((D, S), bf16),
            pltpu.VMEM((S, TQ), f32),
            pltpu.VMEM((S, TQ), f32),
            pltpu.VMEM((2 * D, D), bf16),
            pltpu.VMEM((D, D), bf16),
            pltpu.VMEM((D, F), bf16),
            pltpu.VMEM((F, D), bf16),
            pltpu.SemaphoreType.DMA((3,)),
        ],
        compiler_params=pltpu.CompilerParams(vmem_limit_bytes=110 * 1024 * 1024),
        name="mha_mish_layers",
    )(A_x, A_wqkv, A_wo, B_w1, b1, B_w2)
    return out
```

```python
import functools
import math

import jax
import jax.numpy as jnp
import jax.experimental.pallas as pl
import jax.experimental.pallas.tpu as pltpu

S, D, H, DH, F = 2048, 512, 32, 16, 1792
EPS = 1e-5
QSCALE = (DH ** -0.5) * math.log2(math.e)

TQ = 512
KS = 128
LAG = 3
G = 4
TOKS = 8
UN = 8
SR = KS // G
NQ = S // TQ
NU = H * NQ
NP = S // KS
RB = 256
NRB = S // RB

f32 = jnp.float32
bf16 = jnp.bfloat16


def _ln(x):
    mu = jnp.mean(x, axis=-1, keepdims=True)
    xc = x - mu
    var = jnp.mean(xc * xc, axis=-1, keepdims=True)
    return xc * jax.lax.rsqrt(var + EPS)


def _mish(h):
    sp = jnp.log1p(jnp.exp(-jnp.abs(h))) + jnp.maximum(h, 0.0)
    return h * jnp.tanh(sp)


def _kernel(x_hbm, wqkv_hbm, wo_hbm, w1_hbm, b1_ref, w2_hbm, out_hbm,
            xs_ref, qt_ref, vt_ref, k_ref, ot_ref, sa_ref, sb_ref,
            wqvt_ref, wqkv_ref, wo_ref, w1_ref, w2_ref, xio_ref, sems, xsems):
    def rows(i):
        return pl.ds(pl.multiple_of(i * RB, RB), RB)

    def cp_x(i):
        return pltpu.make_async_copy(x_hbm.at[0, rows(i), :], xio_ref.at[rows(i), :], xsems.at[i])

    def cp_out(i):
        return pltpu.make_async_copy(xio_ref.at[rows(i), :], out_hbm.at[0, rows(i), :], xsems.at[i])

    cp_wo = pltpu.make_async_copy(wo_hbm, wo_ref, sems.at[0])
    cp_w1 = pltpu.make_async_copy(w1_hbm, w1_ref, sems.at[1])
    cp_w2 = pltpu.make_async_copy(w2_hbm, w2_ref, sems.at[2])
    cp_wqkv = pltpu.make_async_copy(wqkv_hbm, wqkv_ref, sems.at[3])
    cp_x(0).start()
    cp_wqkv.start()
    for i in range(1, NRB):
        cp_x(i).start()
    cp_wo.start()
    cp_w1.start()
    cp_w2.start()
    cp_wqkv.wait()
    wqvt_ref[0:D, :] = wqkv_ref[:, 0:D].T
    wqvt_ref[D:2 * D, :] = wqkv_ref[:, 2 * D:3 * D].T

    def st_qkv(i, hb):
        kb = jnp.dot(hb, wqkv_ref[:, D:2 * D], preferred_element_type=f32).astype(bf16)
        for h in range(H):
            k_ref[h, rows(i), :] = kb[:, h * DH:(h + 1) * DH]
        qvt = jax.lax.dot_general(wqvt_ref[...], hb, (((1,), (1,)), ((), ())),
                                  preferred_element_type=f32)
        qt_ref[:, rows(i)] = (qvt[:D] * QSCALE).astype(bf16)
        vt_ref[:, rows(i)] = qvt[D:].astype(bf16)

    def st_in(i):
        cp_x(i).wait()
        x = xio_ref[rows(i), :].astype(f32)
        xs_ref[rows(i), :] = x
        return _ln(x).astype(bf16)

    def st_oproj(i):
        ob = ot_ref[:, rows(i)].T
        x = xs_ref[rows(i), :] + jnp.dot(ob, wo_ref[...], preferred_element_type=f32)
        xs_ref[rows(i), :] = x
        return _ln(x).astype(bf16)

    def st_mlp(i, hb, last):
        h1 = jnp.dot(hb, w1_ref[...], preferred_element_type=f32) + b1_ref[...].astype(f32)
        a = _mish(h1).astype(bf16)
        x = xs_ref[rows(i), :] + jnp.dot(a, w2_ref[...], preferred_element_type=f32)
        if last:
            xio_ref[rows(i), :] = x.astype(xio_ref.dtype)
            cp_out(i).start()
            return None
        xs_ref[rows(i), :] = x
        return _ln(x).astype(bf16)

    def p1_piece(u, j, s_ref, m8, hist):
        h = u // NQ
        qi = u % NQ
        r0 = pl.multiple_of(h * DH, DH)
        q0 = pl.multiple_of(qi * TQ, TQ)
        qt = qt_ref[pl.ds(r0, DH), pl.ds(q0, TQ)]
        s = jnp.dot(k_ref[h, j * KS:(j + 1) * KS, :], qt, preferred_element_type=f32)
        s_ref[j * KS:(j + 1) * KS, :] = s
        for g in range(G):
            for i in range(SR // 8):
                r = g * SR + 8 * i
                m8 = jnp.maximum(m8, s[r:r + 8, :])
            hist.append(m8)
        return m8

    def p2_piece(u, j, s_ref, mfun, l8, acc):
        h = u // NQ
        r0 = pl.multiple_of(h * DH, DH)
        ps = [None] * G
        for gi in range(G):
            g = G - 1 - gi
            r = j * KS + g * SR
            p = jnp.exp2(s_ref[r:r + SR, :] - mfun(gi))
            for i in reversed(range(SR // 8)):
                l8 = l8 + p[8 * i:8 * i + 8, :]
            ps[g] = p.astype(bf16)
        pb = jnp.concatenate(ps, axis=0)
        acc = acc + jnp.dot(vt_ref[pl.ds(r0, DH), j * KS:(j + 1) * KS], pb,
                            preferred_element_type=f32)
        return l8, acc

    def finalize(u, l8, acc):
        l = l8.sum(axis=0, keepdims=True)
        h = u // NQ
        qi = u % NQ
        r0 = pl.multiple_of(h * DH, DH)
        q0 = pl.multiple_of(qi * TQ, TQ)
        ot_ref[pl.ds(r0, DH), pl.ds(q0, TQ)] = (acc / l).astype(bf16)

    def attention():
        minit = jnp.full((8, TQ), -jnp.inf, f32)
        zl = jnp.zeros((8, TQ), f32)
        za = jnp.zeros((DH, TQ), f32)
        m8 = minit
        for j in range(NP):
            m8 = p1_piece(0, j, sa_ref, m8, [])
        sb_ref[(NP - LAG) * KS:, :] = jnp.zeros((LAG * KS, TQ), f32)

        def unit(u, carry, cur_ref, nxt_ref, hist):
            m8_cur, m_prev, l8p, accp = carry
            m = m8_cur.max(axis=0, keepdims=True)
            un = jnp.minimum(u + 1, NU - 1)
            up = jnp.maximum(u - 1, 0)
            m8n = minit
            l8 = zl
            acc = za
            base = len(hist)

            def tok(mm, j):
                def f(gi):
                    idx = base + j * G + gi - TOKS
                    if idx < 0:
                        return mm
                    t = hist[idx][0:1, :]
                    return jnp.maximum(mm, jnp.minimum(mm, t))
                return f

            for j in range(NP):
                m8n = p1_piece(un, j, nxt_ref, m8n, hist)
                if j < LAG:
                    l8p, accp = p2_piece(up, NP - LAG + j, nxt_ref, tok(m_prev, j), l8p, accp)
                    if j == LAG - 1:
                        finalize(up, l8p, accp)
                else:
                    l8, acc = p2_piece(u, j - LAG, cur_ref, tok(m, j), l8, acc)
            return m8n, m, l8, acc

        def group(i, carry):
            hist = []
            for t in range(UN // 2):
                carry = unit(UN * i + 2 * t, carry, sa_ref, sb_ref, hist)
                carry = unit(UN * i + 2 * t + 1, carry, sb_ref, sa_ref, hist)
            return carry

        carry = jax.lax.fori_loop(0, NU // UN, group, (m8, jnp.zeros((1, TQ), f32), zl, za))
        _, m, l8, acc = carry
        for j in range(LAG):
            l8, acc = p2_piece(NU - 1, NP - LAG + j, sb_ref, lambda gi: m, l8, acc)
        finalize(NU - 1, l8, acc)

    def phase_first():
        h = st_in(0)

        def body(i, h):
            hn = st_in(i + 1)
            st_qkv(i, h)
            return hn

        h = jax.lax.fori_loop(0, NRB - 1, body, h)
        st_qkv(NRB - 1, h)

    def phase_mid():
        h2 = st_oproj(0)
        h1 = st_mlp(0, h2, False)
        h2 = st_oproj(1)

        def body(i, carry):
            h2, h1 = carry
            h1n = st_mlp(i, h2, False)
            h2n = st_oproj(i + 1)
            st_qkv(i - 1, h1)
            return h2n, h1n

        h2, h1 = jax.lax.fori_loop(1, NRB - 1, body, (h2, h1))
        h1n = st_mlp(NRB - 1, h2, False)
        st_qkv(NRB - 2, h1)
        st_qkv(NRB - 1, h1n)

    def phase_last():
        h2 = st_oproj(0)

        def body(i, h2):
            st_mlp(i, h2, True)
            return st_oproj(i + 1)

        h2 = jax.lax.fori_loop(0, NRB - 1, body, h2)
        st_mlp(NRB - 1, h2, True)

    phase_first()
    attention()
    cp_wo.wait()
    cp_w1.wait()
    cp_w2.wait()
    phase_mid()
    attention()
    phase_last()
    for i in range(NRB):
        cp_out(i).wait()


@jax.jit
def pallas_interleave_layers__mha_block__dense_activation_mish__prompt_kernel(
    A_x: jax.Array,
    A_wqkv: jax.Array,
    A_wo: jax.Array,
    B_x: jax.Array,
    B_w1: jax.Array,
    B_b1: jax.Array,
    B_w2: jax.Array,
):
    b1 = B_b1.reshape(1, F)
    vmem = pl.BlockSpec(memory_space=pltpu.VMEM)
    hbm = pl.BlockSpec(memory_space=pl.ANY)
    out = pl.pallas_call(
        _kernel,
        out_shape=jax.ShapeDtypeStruct((1, S, D), A_x.dtype),
        in_specs=[hbm, hbm, hbm, hbm, vmem, hbm],
        out_specs=hbm,
        scratch_shapes=[
            pltpu.VMEM((S, D), f32),
            pltpu.VMEM((D, S), bf16),
            pltpu.VMEM((D, S), bf16),
            pltpu.VMEM((H, S, DH), bf16),
            pltpu.VMEM((D, S), bf16),
            pltpu.VMEM((S, TQ), f32),
            pltpu.VMEM((S, TQ), f32),
            pltpu.VMEM((2 * D, D), bf16),
            pltpu.VMEM((D, 3 * D), bf16),
            pltpu.VMEM((D, D), bf16),
            pltpu.VMEM((D, F), bf16),
            pltpu.VMEM((F, D), bf16),
            pltpu.VMEM((S, D), bf16),
            pltpu.SemaphoreType.DMA((4,)),
            pltpu.SemaphoreType.DMA((NRB,)),
        ],
        compiler_params=pltpu.CompilerParams(vmem_limit_bytes=110 * 1024 * 1024),
        name="mha_mish_layers",
    )(A_x, A_wqkv, A_wo, B_w1, b1, B_w2)
    return out
```

```python
import functools
import math

import jax
import jax.numpy as jnp
import jax.experimental.pallas as pl
import jax.experimental.pallas.tpu as pltpu

S, D, H, DH, F = 2048, 512, 32, 16, 1792
EPS = 1e-5
QSCALE = (DH ** -0.5) * math.log2(math.e)

TQ = 512
KS = 128
LAG = 3
G = 4
TOKS = 8
UN = 8
SR = KS // G
NQ = S // TQ
NU = H * NQ
NP = S // KS
RB = 256
NRB = S // RB

f32 = jnp.float32
bf16 = jnp.bfloat16


def _ln(x):
    mu = jnp.mean(x, axis=-1, keepdims=True)
    xc = x - mu
    var = jnp.mean(xc * xc, axis=-1, keepdims=True)
    return xc * jax.lax.rsqrt(var + EPS)


def _mish(h):
    sp = jnp.log1p(jnp.exp(-jnp.abs(h))) + jnp.maximum(h, 0.0)
    return h * jnp.tanh(sp)


def _kernel(x_hbm, wqkv_hbm, wo_hbm, w1_hbm, b1_ref, w2_hbm, out_hbm,
            xs_ref, qt_ref, vt_ref, k_ref, ot_ref, sa_ref, sb_ref,
            wqvt_ref, wqkv_ref, wo_ref, w1_ref, w2_ref, xio_ref, sems, xsems):
    def rows(i):
        return pl.ds(pl.multiple_of(i * RB, RB), RB)

    def cp_x(i):
        return pltpu.make_async_copy(x_hbm.at[0, rows(i), :], xio_ref.at[rows(i), :], xsems.at[i])

    def cp_out(i):
        return pltpu.make_async_copy(xio_ref.at[rows(i), :], out_hbm.at[0, rows(i), :], xsems.at[i])

    cp_wo = pltpu.make_async_copy(wo_hbm, wo_ref, sems.at[0])
    cp_w1 = pltpu.make_async_copy(w1_hbm, w1_ref, sems.at[1])
    cp_w2 = pltpu.make_async_copy(w2_hbm, w2_ref, sems.at[2])
    cp_wqkv = pltpu.make_async_copy(wqkv_hbm, wqkv_ref, sems.at[3])
    cp_x(0).start()
    cp_wqkv.start()
    for i in range(1, NRB):
        cp_x(i).start()
    cp_wo.start()
    cp_w1.start()
    cp_w2.start()
    cp_wqkv.wait()
    wqvt_ref[0:D, :] = wqkv_ref[:, 0:D].T
    wqvt_ref[D:2 * D, :] = wqkv_ref[:, 2 * D:3 * D].T

    def st_qkv(i, hb):
        kb = jnp.dot(hb, wqkv_ref[:, D:2 * D], preferred_element_type=f32).astype(bf16)
        for h in range(H):
            k_ref[h, rows(i), :] = kb[:, h * DH:(h + 1) * DH]
        qvt = jax.lax.dot_general(wqvt_ref[...], hb, (((1,), (1,)), ((), ())),
                                  preferred_element_type=f32)
        qt_ref[:, rows(i)] = (qvt[:D] * QSCALE).astype(bf16)
        vt_ref[:, rows(i)] = qvt[D:].astype(bf16)

    def st_in(i):
        cp_x(i).wait()
        x = xio_ref[rows(i), :].astype(f32)
        xs_ref[rows(i), :] = x
        return _ln(x).astype(bf16)

    def st_oproj(i):
        ob = ot_ref[:, rows(i)].T
        x = xs_ref[rows(i), :] + jnp.dot(ob, wo_ref[...], preferred_element_type=f32)
        xs_ref[rows(i), :] = x
        return _ln(x).astype(bf16)

    def st_mlp(i, hb, last, mid=None):
        h1 = jnp.dot(hb, w1_ref[...], preferred_element_type=f32) + b1_ref[...].astype(f32)
        a = _mish(h1).astype(bf16)
        if mid is not None:
            mid()
        x = xs_ref[rows(i), :] + jnp.dot(a, w2_ref[...], preferred_element_type=f32)
        if last:
            xio_ref[rows(i), :] = x.astype(xio_ref.dtype)
            cp_out(i).start()
            return None
        xs_ref[rows(i), :] = x
        return _ln(x).astype(bf16)

    def p1_piece(u, j, s_ref, m8, hist):
        h = u // NQ
        qi = u % NQ
        r0 = pl.multiple_of(h * DH, DH)
        q0 = pl.multiple_of(qi * TQ, TQ)
        qt = qt_ref[pl.ds(r0, DH), pl.ds(q0, TQ)]
        s = jnp.dot(k_ref[h, j * KS:(j + 1) * KS, :], qt, preferred_element_type=f32)
        s_ref[j * KS:(j + 1) * KS, :] = s
        for g in range(G):
            for i in range(SR // 8):
                r = g * SR + 8 * i
                m8 = jnp.maximum(m8, s[r:r + 8, :])
            hist.append(m8)
        return m8

    def p2_piece(u, j, s_ref, mfun, l8, acc):
        h = u // NQ
        r0 = pl.multiple_of(h * DH, DH)
        ps = [None] * G
        for gi in range(G):
            g = G - 1 - gi
            r = j * KS + g * SR
            p = jnp.exp2(s_ref[r:r + SR, :] - mfun(gi))
            for i in reversed(range(SR // 8)):
                l8 = l8 + p[8 * i:8 * i + 8, :]
            ps[g] = p.astype(bf16)
        pb = jnp.concatenate(ps, axis=0)
        acc = acc + jnp.dot(vt_ref[pl.ds(r0, DH), j * KS:(j + 1) * KS], pb,
                            preferred_element_type=f32)
        return l8, acc

    def finalize(u, l8, acc):
        l = l8.sum(axis=0, keepdims=True)
        h = u // NQ
        qi = u % NQ
        r0 = pl.multiple_of(h * DH, DH)
        q0 = pl.multiple_of(qi * TQ, TQ)
        ot_ref[pl.ds(r0, DH), pl.ds(q0, TQ)] = (acc / l).astype(bf16)

    def attention():
        minit = jnp.full((8, TQ), -jnp.inf, f32)
        zl = jnp.zeros((8, TQ), f32)
        za = jnp.zeros((DH, TQ), f32)
        m8 = minit
        for j in range(NP):
            m8 = p1_piece(0, j, sa_ref, m8, [])
        sb_ref[(NP - LAG) * KS:, :] = jnp.zeros((LAG * KS, TQ), f32)

        def unit(u, carry, cur_ref, nxt_ref, hist):
            m8_cur, m_prev, l8p, accp = carry
            m = m8_cur.max(axis=0, keepdims=True)
            un = jnp.minimum(u + 1, NU - 1)
            up = jnp.maximum(u - 1, 0)
            m8n = minit
            l8 = zl
            acc = za
            base = len(hist)

            def tok(mm, j):
                def f(gi):
                    idx = base + j * G + gi - TOKS
                    if idx < 0:
                        return mm
                    t = hist[idx][0:1, :]
                    return jnp.maximum(mm, jnp.minimum(mm, t))
                return f

            for j in range(NP):
                m8n = p1_piece(un, j, nxt_ref, m8n, hist)
                if j < LAG:
                    l8p, accp = p2_piece(up, NP - LAG + j, nxt_ref, tok(m_prev, j), l8p, accp)
                    if j == LAG - 1:
                        finalize(up, l8p, accp)
                else:
                    l8, acc = p2_piece(u, j - LAG, cur_ref, tok(m, j), l8, acc)
            return m8n, m, l8, acc

        def group(i, carry):
            hist = []
            for t in range(UN // 2):
                carry = unit(UN * i + 2 * t, carry, sa_ref, sb_ref, hist)
                carry = unit(UN * i + 2 * t + 1, carry, sb_ref, sa_ref, hist)
            return carry

        carry = jax.lax.fori_loop(0, NU // UN, group, (m8, jnp.zeros((1, TQ), f32), zl, za))
        _, m, l8, acc = carry
        for j in range(LAG):
            l8, acc = p2_piece(NU - 1, NP - LAG + j, sb_ref, lambda gi: m, l8, acc)
        finalize(NU - 1, l8, acc)

    def phase_first():
        h = st_in(0)

        def body(i, h):
            hn = st_in(i + 1)
            st_qkv(i, h)
            return hn

        h = jax.lax.fori_loop(0, NRB - 1, body, h)
        st_qkv(NRB - 1, h)

    def phase_mid():
        box = []
        h1 = st_mlp(0, st_oproj(0), False, lambda: box.append(st_oproj(1)))
        h2 = box[0]

        def body(i, carry):
            h2, h1 = carry
            box = []
            h1n = st_mlp(i, h2, False, lambda: box.append(st_oproj(i + 1)))
            st_qkv(i - 1, h1)
            return box[0], h1n

        h2, h1 = jax.lax.fori_loop(1, NRB - 1, body, (h2, h1))
        h1n = st_mlp(NRB - 1, h2, False)
        st_qkv(NRB - 2, h1)
        st_qkv(NRB - 1, h1n)

    def phase_last():
        h2 = st_oproj(0)

        def body(i, h2):
            box = []
            st_mlp(i, h2, True, lambda: box.append(st_oproj(i + 1)))
            return box[0]

        h2 = jax.lax.fori_loop(0, NRB - 1, body, h2)
        st_mlp(NRB - 1, h2, True)

    phase_first()
    attention()
    cp_wo.wait()
    cp_w1.wait()
    cp_w2.wait()
    phase_mid()
    attention()
    phase_last()
    for i in range(NRB):
        cp_out(i).wait()


@jax.jit
def pallas_interleave_layers__mha_block__dense_activation_mish__prompt_kernel(
    A_x: jax.Array,
    A_wqkv: jax.Array,
    A_wo: jax.Array,
    B_x: jax.Array,
    B_w1: jax.Array,
    B_b1: jax.Array,
    B_w2: jax.Array,
):
    b1 = B_b1.reshape(1, F)
    vmem = pl.BlockSpec(memory_space=pltpu.VMEM)
    hbm = pl.BlockSpec(memory_space=pl.ANY)
    out = pl.pallas_call(
        _kernel,
        out_shape=jax.ShapeDtypeStruct((1, S, D), A_x.dtype),
        in_specs=[hbm, hbm, hbm, hbm, vmem, hbm],
        out_specs=hbm,
        scratch_shapes=[
            pltpu.VMEM((S, D), f32),
            pltpu.VMEM((D, S), bf16),
            pltpu.VMEM((D, S), bf16),
            pltpu.VMEM((H, S, DH), bf16),
            pltpu.VMEM((D, S), bf16),
            pltpu.VMEM((S, TQ), f32),
            pltpu.VMEM((S, TQ), f32),
            pltpu.VMEM((2 * D, D), bf16),
            pltpu.VMEM((D, 3 * D), bf16),
            pltpu.VMEM((D, D), bf16),
            pltpu.VMEM((D, F), bf16),
            pltpu.VMEM((F, D), bf16),
            pltpu.VMEM((S, D), bf16),
            pltpu.SemaphoreType.DMA((4,)),
            pltpu.SemaphoreType.DMA((NRB,)),
        ],
        compiler_params=pltpu.CompilerParams(vmem_limit_bytes=110 * 1024 * 1024),
        name="mha_mish_layers",
    )(A_x, A_wqkv, A_wo, B_w1, b1, B_w2)
    return out
```

```python
import math

import jax
import jax.numpy as jnp
import jax.experimental.pallas as pl
import jax.experimental.pallas.tpu as pltpu

S, D, H, DH, F = 2048, 512, 32, 16, 1792
EPS = 1e-5
QSCALE = (DH ** -0.5) * math.log2(math.e)

TQ = 512
KS = 128
LAG = 3
G = 4
TOKS = 8
UN = 8
SR = KS // G
NQ = S // TQ
NU = H * NQ
NP = S // KS
RB = 256
NRB = S // RB

f32 = jnp.float32
bf16 = jnp.bfloat16


def _ln(x):
    mu = jnp.mean(x, axis=-1, keepdims=True)
    xc = x - mu
    var = jnp.mean(xc * xc, axis=-1, keepdims=True)
    return xc * jax.lax.rsqrt(var + EPS)


def _mish(h):
    sp = jnp.log1p(jnp.exp(-jnp.abs(h))) + jnp.maximum(h, 0.0)
    return h * jnp.tanh(sp)


def _kernel(x_hbm, wqkv_hbm, wo_hbm, w1_hbm, b1_ref, w2_hbm, out_hbm,
            xs_ref, qt_ref, vt_ref, k_ref, ot_ref, sa_ref, sb_ref,
            wqvt_ref, wqkv_ref, wo_ref, w1_ref, w2_ref, xio_ref, sems, xsems):
    def rows(i):
        return pl.ds(pl.multiple_of(i * RB, RB), RB)

    def cp_x(i):
        return pltpu.make_async_copy(x_hbm.at[0, rows(i), :], xio_ref.at[rows(i), :], xsems.at[i])

    def cp_out(i):
        return pltpu.make_async_copy(xio_ref.at[rows(i), :], out_hbm.at[0, rows(i), :], xsems.at[i])

    cp_wo = pltpu.make_async_copy(wo_hbm, wo_ref, sems.at[0])
    cp_w1 = pltpu.make_async_copy(w1_hbm, w1_ref, sems.at[1])
    cp_w2 = pltpu.make_async_copy(w2_hbm, w2_ref, sems.at[2])
    cp_w = [pltpu.make_async_copy(wqkv_hbm.at[:, c * D:(c + 1) * D],
                                  wqkv_ref.at[:, c * D:(c + 1) * D], sems.at[3 + c])
            for c in range(3)]
    cp_w[0].start()
    cp_x(0).start()
    cp_w[2].start()
    cp_w[1].start()
    for i in range(1, NRB):
        cp_x(i).start()
    cp_wo.start()
    cp_w1.start()
    cp_w2.start()

    def st_qkv(i, hb):
        kb = jnp.dot(hb, wqkv_ref[:, D:2 * D], preferred_element_type=f32).astype(bf16)
        for h in range(H):
            k_ref[h, rows(i), :] = kb[:, h * DH:(h + 1) * DH]
        qvt = jax.lax.dot_general(wqvt_ref[...], hb, (((1,), (1,)), ((), ())),
                                  preferred_element_type=f32)
        qt_ref[:, rows(i)] = (qvt[:D] * QSCALE).astype(bf16)
        vt_ref[:, rows(i)] = qvt[D:].astype(bf16)

    def st_in(i):
        cp_x(i).wait()
        x = xio_ref[rows(i), :].astype(f32)
        xs_ref[rows(i), :] = x
        return _ln(x).astype(bf16)

    def st_oproj(i):
        ob = ot_ref[:, rows(i)].T
        x = xs_ref[rows(i), :] + jnp.dot(ob, wo_ref[...], preferred_element_type=f32)
        xs_ref[rows(i), :] = x
        return _ln(x).astype(bf16)

    def st_mlp(i, hb, last, mid=None):
        h1 = jnp.dot(hb, w1_ref[...], preferred_element_type=f32) + b1_ref[...].astype(f32).reshape(1, F)
        a = _mish(h1).astype(bf16)
        if mid is not None:
            mid()
        x = xs_ref[rows(i), :] + jnp.dot(a, w2_ref[...], preferred_element_type=f32)
        if last:
            xio_ref[rows(i), :] = x.astype(xio_ref.dtype)
            cp_out(i).start()
            return None
        xs_ref[rows(i), :] = x
        return _ln(x).astype(bf16)

    def p1_piece(u, j, s_ref, m8, hist):
        h = u // NQ
        qi = u % NQ
        r0 = pl.multiple_of(h * DH, DH)
        q0 = pl.multiple_of(qi * TQ, TQ)
        qt = qt_ref[pl.ds(r0, DH), pl.ds(q0, TQ)]
        s = jnp.dot(k_ref[h, j * KS:(j + 1) * KS, :], qt, preferred_element_type=f32)
        s_ref[j * KS:(j + 1) * KS, :] = s
        for g in range(G):
            for i in range(SR // 8):
                r = g * SR + 8 * i
                m8 = jnp.maximum(m8, s[r:r + 8, :])
            hist.append(m8)
        return m8

    def p2_piece(u, j, s_ref, mfun, l8, acc):
        h = u // NQ
        r0 = pl.multiple_of(h * DH, DH)
        ps = [None] * G
        for gi in range(G):
            g = G - 1 - gi
            r = j * KS + g * SR
            p = jnp.exp2(s_ref[r:r + SR, :] - mfun(gi))
            for i in reversed(range(SR // 8)):
                l8 = l8 + p[8 * i:8 * i + 8, :]
            ps[g] = p.astype(bf16)
        pb = jnp.concatenate(ps, axis=0)
        acc = acc + jnp.dot(vt_ref[pl.ds(r0, DH), j * KS:(j + 1) * KS], pb,
                            preferred_element_type=f32)
        return l8, acc

    def finalize(u, l8, acc):
        l = l8.sum(axis=0, keepdims=True)
        h = u // NQ
        qi = u % NQ
        r0 = pl.multiple_of(h * DH, DH)
        q0 = pl.multiple_of(qi * TQ, TQ)
        ot_ref[pl.ds(r0, DH), pl.ds(q0, TQ)] = (acc / l).astype(bf16)

    def attention():
        minit = jnp.full((8, TQ), -jnp.inf, f32)
        zl = jnp.zeros((8, TQ), f32)
        za = jnp.zeros((DH, TQ), f32)
        m8 = minit
        for j in range(NP):
            m8 = p1_piece(0, j, sa_ref, m8, [])
        sb_ref[(NP - LAG) * KS:, :] = jnp.zeros((LAG * KS, TQ), f32)

        def unit(u, carry, cur_ref, nxt_ref, hist):
            m8_cur, m_prev, l8p, accp = carry
            m = m8_cur.max(axis=0, keepdims=True)
            un = jnp.minimum(u + 1, NU - 1)
            up = jnp.maximum(u - 1, 0)
            m8n = minit
            l8 = zl
            acc = za
            base = len(hist)

            def tok(mm, j):
                def f(gi):
                    idx = base + j * G + gi - TOKS
                    if idx < 0:
                        return mm
                    t = hist[idx][0:1, :]
                    return jnp.maximum(mm, jnp.minimum(mm, t))
                return f

            for j in range(NP):
                m8n = p1_piece(un, j, nxt_ref, m8n, hist)
                if j < LAG:
                    l8p, accp = p2_piece(up, NP - LAG + j, nxt_ref, tok(m_prev, j), l8p, accp)
                    if j == LAG - 1:
                        finalize(up, l8p, accp)
                else:
                    l8, acc = p2_piece(u, j - LAG, cur_ref, tok(m, j), l8, acc)
            return m8n, m, l8, acc

        def group(i, carry):
            hist = []
            for t in range(UN // 2):
                carry = unit(UN * i + 2 * t, carry, sa_ref, sb_ref, hist)
                carry = unit(UN * i + 2 * t + 1, carry, sb_ref, sa_ref, hist)
            return carry

        carry = jax.lax.fori_loop(0, NU // UN, group, (m8, jnp.zeros((1, TQ), f32), zl, za))
        _, m, l8, acc = carry
        for j in range(LAG):
            l8, acc = p2_piece(NU - 1, NP - LAG + j, sb_ref, lambda gi: m, l8, acc)
        finalize(NU - 1, l8, acc)

    def phase_first():
        cp_w[0].wait()
        wqvt_ref[0:D, :] = wqkv_ref[:, 0:D].T
        h = st_in(0)
        cp_w[2].wait()
        wqvt_ref[D:2 * D, :] = wqkv_ref[:, 2 * D:3 * D].T
        cp_w[1].wait()

        def body(i, h):
            hn = st_in(i + 1)
            st_qkv(i, h)
            return hn

        h = jax.lax.fori_loop(0, NRB - 1, body, h)
        st_qkv(NRB - 1, h)

    def phase_mid():
        box = []
        h1 = st_mlp(0, st_oproj(0), False, lambda: box.append(st_oproj(1)))
        h2 = box[0]

        def body(i, carry):
            h2, h1 = carry
            box = []
            h1n = st_mlp(i, h2, False, lambda: box.append(st_oproj(i + 1)))
            st_qkv(i - 1, h1)
            return box[0], h1n

        h2, h1 = jax.lax.fori_loop(1, NRB - 1, body, (h2, h1))
        h1n = st_mlp(NRB - 1, h2, False)
        st_qkv(NRB - 2, h1)
        st_qkv(NRB - 1, h1n)

    def phase_last():
        h2 = st_oproj(0)

        def body(i, h2):
            box = []
            st_mlp(i, h2, True, lambda: box.append(st_oproj(i + 1)))
            return box[0]

        h2 = jax.lax.fori_loop(0, NRB - 1, body, h2)
        st_mlp(NRB - 1, h2, True)

    phase_first()
    attention()
    cp_wo.wait()
    cp_w1.wait()
    cp_w2.wait()
    phase_mid()
    attention()
    phase_last()
    for i in range(NRB):
        cp_out(i).wait()


@jax.jit
def pallas_interleave_layers__mha_block__dense_activation_mish__prompt_kernel(
    A_x: jax.Array,
    A_wqkv: jax.Array,
    A_wo: jax.Array,
    B_x: jax.Array,
    B_w1: jax.Array,
    B_b1: jax.Array,
    B_w2: jax.Array,
):
    b1 = B_b1
    vmem = pl.BlockSpec(memory_space=pltpu.VMEM)
    hbm = pl.BlockSpec(memory_space=pl.ANY)
    out = pl.pallas_call(
        _kernel,
        out_shape=jax.ShapeDtypeStruct((1, S, D), A_x.dtype),
        in_specs=[hbm, hbm, hbm, hbm, vmem, hbm],
        out_specs=hbm,
        scratch_shapes=[
            pltpu.VMEM((S, D), f32),
            pltpu.VMEM((D, S), bf16),
            pltpu.VMEM((D, S), bf16),
            pltpu.VMEM((H, S, DH), bf16),
            pltpu.VMEM((D, S), bf16),
            pltpu.VMEM((S, TQ), f32),
            pltpu.VMEM((S, TQ), f32),
            pltpu.VMEM((2 * D, D), bf16),
            pltpu.VMEM((D, 3 * D), bf16),
            pltpu.VMEM((D, D), bf16),
            pltpu.VMEM((D, F), bf16),
            pltpu.VMEM((F, D), bf16),
            pltpu.VMEM((S, D), bf16),
            pltpu.SemaphoreType.DMA((6,)),
            pltpu.SemaphoreType.DMA((NRB,)),
        ],
        compiler_params=pltpu.CompilerParams(vmem_limit_bytes=96 * 1024 * 1024),
        name="mha_mish_layers",
    )(A_x, A_wqkv, A_wo, B_w1, b1, B_w2)
    return out
```
